```python
import jax
import jax.numpy as jnp

def _softmax(x, axis=-1):
    return jax.nn.softmax(x, axis=axis)

def _gelu(x):
    return jax.nn.gelu(x, approximate=True)

def _silu(x):
    return jax.nn.silu(x)

def _sigmoid(x):
    return jax.nn.sigmoid(x)

def _layernorm(x, axis=-1, eps=1e-05):
    m = jnp.mean(x, axis=axis, keepdims=True)
    v = jnp.var(x, axis=axis, keepdims=True)
    return (x - m) / jnp.sqrt(v + eps)

def _scatter_add(tgt, idx, src, axis=0):
    return tgt.at[idx].add(src)

def _segment_sum(src, seg, n):
    return jax.ops.segment_sum(src, seg, n)

class _Rng:

    def __init__(self, key):
        self._k = key

    def _next(self):
        self._k, sub = jax.random.split(self._k)
        return sub

    def normal(self, shape):
        return jax.random.normal(self._next(), shape, dtype=jnp.bfloat16)

    def randint(self, lo, hi, shape):
        return jax.random.randint(self._next(), shape, lo, hi, dtype=jnp.int32)

    def uniform(self, shape, lo=0.0, hi=1.0):
        return jax.random.uniform(self._next(), shape, jnp.bfloat16, lo, hi)

    def permutation(self, n):
        return jax.random.permutation(self._next(), n)
kernel_name = 'sequential_preLN__memory_aug_recurrent_mem_tr__moe_arch_mod__prompt'

def setup_inputs():
    _rng = _Rng(jax.random.key(int.from_bytes(__import__("os").urandom(4), "little")))
    _w = lambda a: (lambda t: t.astype(jnp.bfloat16) if jnp.issubdtype(t.dtype, jnp.floating) else t)(jnp.asarray(a))

    def _A_setup():
        B, S, Dm = (1, 2048, 512)
        H, Dh = (32, 128)
        M, seg = (8, 32)
        seg = min(seg, S)
        S = S // seg * seg
        return {'x': _w((lambda *s: _rng.normal(s) * 0.05)(B, S, Dm)), 'mem0': _w((lambda *s: _rng.normal(s) * 0.05)(B, M, Dm)), 'Wq': _w((lambda *s: _rng.normal(s) * 0.05)(Dm, H, Dh) * Dm ** (-0.5)), 'Wk': _w((lambda *s: _rng.normal(s) * 0.05)(Dm, H, Dh) * Dm ** (-0.5)), 'Wv': _w((lambda *s: _rng.normal(s) * 0.05)(Dm, H, Dh) * Dm ** (-0.5)), 'Wo': _w((lambda *s: _rng.normal(s) * 0.05)(H, Dh, Dm) * (H * Dh) ** (-0.5)), 'seg_len': seg}
    _A_in = _A_setup()

    def _B_setup():
        B, S, D, F, C = (1, 2048, 512, 1792, 2)
        return {'x': _w((lambda *s: _rng.normal(s) * 0.05)(B, S, D)), 'w_r': _w((lambda *s: _rng.normal(s) * 0.05)(D)), 'w_gate': _w((lambda *s: _rng.normal(s) * 0.05)(D, F)), 'w_up': _w((lambda *s: _rng.normal(s) * 0.05)(D, F)), 'w_down': _w((lambda *s: _rng.normal(s) * 0.05)(F, D))}
    _B_in = _B_setup()
    return {'A_x': _A_in['x'], 'A_mem0': _A_in['mem0'], 'A_Wq': _A_in['Wq'], 'A_Wk': _A_in['Wk'], 'A_Wv': _A_in['Wv'], 'A_Wo': _A_in['Wo'], 'A_seg_len': _A_in['seg_len'], 'B_x': _B_in['x'], 'B_w_r': _B_in['w_r'], 'B_w_gate': _B_in['w_gate'], 'B_w_up': _B_in['w_up'], 'B_w_down': _B_in['w_down']}

def reference(A_x, A_mem0, A_Wq, A_Wk, A_Wv, A_Wo, A_seg_len, B_x, B_w_r, B_w_gate, B_w_up, B_w_down):

    def _A_ref(x, mem0, Wq, Wk, Wv, Wo, seg_len):
        B, S, Dm = x.shape
        H, Dh = (Wq.shape[1], Wq.shape[2])
        M = mem0.shape[1]
        scale = Dh ** (-0.5)
        n_seg = S // seg_len
        L = M + seg_len
        idx = jnp.arange(L)
        mask = (idx[:, None] < M) | (idx[:, None] >= idx[None, :])
        mem = mem0
        outs = []
        for s in range(n_seg):
            xs = x[:, s * seg_len:(s + 1) * seg_len, :].copy()
            h = jnp.concatenate([mem, xs], axis=1)
            q = jnp.einsum('btd,dhe->bhte', h, Wq)
            k = jnp.einsum('btd,dhe->bhte', h, Wk)
            v = jnp.einsum('btd,dhe->bhte', h, Wv)
            scores = jnp.einsum('bhqe,bhke->bhqk', q, k) * scale
            scores = jnp.where(mask[None, None], scores, -1000000000.0)
            p = _softmax(scores, axis=-1)
            o = jnp.einsum('bhqk,bhke->bhqe', p, v)
            o = jnp.einsum('bhte,hed->btd', o, Wo)
            mem = o[:, :M, :].copy()
            outs.append(o[:, M:, :])
        return jnp.concatenate(outs, axis=1)

    def _B_ref(x, w_r, w_gate, w_up, w_down):
        B, S, D = x.shape
        C = 2
        r = x @ w_r
        idx = jnp.argsort(-r, axis=-1)[:, :C]
        idx_e = jnp.repeat(idx.reshape(B, C, 1), D, axis=2)
        x_sel = jnp.take_along_axis(x, idx_e, axis=1)
        g = _silu(x_sel @ w_gate)
        u = x_sel @ w_up
        y = g * u @ w_down
        r_sel = _sigmoid(jnp.take_along_axis(r, idx, axis=1))
        y = y * r_sel.reshape(B, C, 1)
        b_off = (jnp.arange(B) * S).reshape(B, 1)
        flat_idx = (idx + b_off).reshape(B * C)
        zero = (x * 0.0).reshape(B * S, D)
        upd = _scatter_add(zero, flat_idx, y.reshape(B * C, D), axis=0)
        return x + upd.reshape(B, S, D)
    x = A_x
    h = x + _A_ref(_layernorm(x, axis=-1), A_mem0, A_Wq, A_Wk, A_Wv, A_Wo, A_seg_len)
    h2 = h + _B_ref(_layernorm(h, axis=-1), B_w_r, B_w_gate, B_w_up, B_w_down)
    return h2
```

```python
import functools
import math

import jax
import jax.numpy as jnp
import numpy as np
from jax import lax
from jax.experimental import pallas as pl
from jax.experimental.pallas import tpu as pltpu

F32, BF16, U32, I32 = jnp.float32, jnp.bfloat16, jnp.uint32, jnp.int32
NN = (((1,), (0,)), ((), ()))
NT = (((1,), (1,)), ((), ()))
LANES = 128
PRE = 8
GROUP = 4
EPS_BF16 = float(np.float32(1e-05).astype(BF16))
LOG2E = math.log2(math.e)
INT_MIN = int(np.iinfo(np.int32).min)


def _rb(x):
    return x.astype(BF16).astype(F32)


def _layernorm(x):
    inv_n = 1.0 / x.shape[-1]
    m = jnp.sum(x, axis=-1, keepdims=True) * inv_n
    c = x - m
    v = _rb(jnp.sum(c * c, axis=-1, keepdims=True) * inv_n)
    d = _rb(jnp.sqrt(_rb(v + EPS_BF16)))
    return _rb(_rb(x - _rb(m)) * (1.0 / d))


def _dot(a, b, dims=NN):
    return lax.dot_general(a, b, dims, preferred_element_type=F32)


def _kernel(x_hbm, mem_hbm, wq_hbm, wk_hbm, wv_hbm, wo_hbm, wr_hbm, wg_hbm,
            wu_hbm, wd_hbm, out_hbm,
            x_v, xpre_v, lpre_v, raw_v, w_v, wo_v, pre_v, mem_v, wr_v, wg_v,
            wu_v, wd_v, ob_v, xn_v, att_v, h_v, out_v, r_v, patch_v,
            sem_raw, sem, *, n_seg, seg, n_mem, n_head, d_model):
    live = seg - PRE
    rows = n_mem + seg
    n_pair = n_head // 2
    n_col = d_model // LANES
    w_hbms = (wq_hbm, wk_hbm, wv_hbm)

    def raw_copy(t, j):
        return pltpu.make_async_copy(
            w_hbms[t].bitcast(U32).at[:, j, :], raw_v.at[t, j], sem_raw.at[t, j])

    cp_xpre = pltpu.make_async_copy(x_hbm.at[:, pl.ds(live, PRE), :], xpre_v, sem.at[0])
    cp_mem = pltpu.make_async_copy(mem_hbm, mem_v, sem.at[1])
    cp_wr = pltpu.make_async_copy(wr_hbm, wr_v, sem.at[2])
    cp_x = pltpu.make_async_copy(x_hbm, x_v, sem.at[3])
    cp_wg = pltpu.make_async_copy(wg_hbm, wg_v, sem.at[4])
    cp_wu = pltpu.make_async_copy(wu_hbm, wu_v, sem.at[5])
    cp_wd = pltpu.make_async_copy(wd_hbm, wd_v, sem.at[6])
    cp_wo = [pltpu.make_async_copy(
        wo_hbm.bitcast(U32).at[:, pl.ds(n * LANES, LANES)], wo_v.at[n], sem.at[11 + n])
        for n in range(n_col)]

    cp_xpre.start()
    for j in range(n_pair):
        for t in range(3):
            raw_copy(t, j).start()
    cp_mem.start()
    cp_wr.start()
    for c in cp_wo:
        c.start()
    cp_x.start()

    cp_xpre.wait()
    xp = xpre_v[...].astype(F32).reshape(n_seg * PRE, d_model)
    lpre_v[...] = _layernorm(xp).astype(BF16)

    def pro_body(j, carry):
        for t in range(3):
            raw_copy(t, j).wait()
        for t in range(3):
            a = raw_v[t, j, pl.ds(0, d_model // 2, stride=2), :]
            b = raw_v[t, j, pl.ds(1, d_model // 2, stride=2), :]
            for p, w in enumerate(((a & 0xFFFF) | (b << 16),
                                   (a >> 16) | (b & np.uint32(0xFFFF0000)))):
                w_v[t, 2 * j + p] = w
                pre_v[t, 2 * j + p] = _dot(lpre_v[...], pltpu.bitcast(w, BF16))
        return carry

    lax.fori_loop(0, n_pair, pro_body, 0)

    cp_mem.wait()
    cp_wr.wait()
    cp_x.wait()
    for c in cp_wo:
        c.wait()
    cp_wg.start()
    cp_wu.start()
    cp_wd.start()

    def norm_live(s):
        xn_v[...] = _layernorm(x_v[s].astype(F32)[:live])

    seg_lane = lax.broadcasted_iota(I32, (seg, LANES), 1)

    def finish(s, slot):
        h = _rb(x_v[slot].astype(F32) + _rb(att_v[...]))
        hn = _layernorm(h)
        h_v[pl.ds(pl.multiple_of(slot * seg, seg), seg), :] = h
        out_v[slot] = (h + hn).astype(BF16)
        wr = wr_v[...].astype(F32)
        r = _rb(jnp.sum(hn * wr, axis=-1, keepdims=True))
        r_v[...] = jnp.where(seg_lane == s, r, r_v[...])

    norm_live(0)
    att_v[...] = jnp.zeros_like(att_v)
    r_v[...] = jnp.zeros_like(r_v)

    row = lax.broadcasted_iota(I32, (rows, rows), 0)
    col = lax.broadcasted_iota(I32, (rows, rows), 1)
    mask = (row < n_mem) | (row >= col)
    cut = n_seg - 8
    cp_out0 = pltpu.make_async_copy(out_v.at[pl.ds(0, cut)], out_hbm.at[pl.ds(0, cut)], sem.at[7])
    cp_out1 = pltpu.make_async_copy(out_v.at[pl.ds(cut, n_seg - cut)],
                                    out_hbm.at[pl.ds(cut, n_seg - cut)], sem.at[8])

    def seg_body(s, mem):
        @pl.when(s == cut + 1)
        def _():
            cp_out0.start()

        lhs = jnp.concatenate([mem, xn_v[...]], axis=0).astype(BF16)
        pre_rows = pl.ds(pl.multiple_of(s * PRE, PRE), PRE)
        q, k, v, p, l = {}, {}, {}, {}, {}
        acc = [None] * n_col

        def proj(h):
            for t, dst in enumerate((q, k, v)):
                dst[h] = jnp.concatenate(
                    [_dot(lhs, pltpu.bitcast(w_v[t, h], BF16)), pre_v[t, h, pre_rows, :]], axis=0)

        def scores(h):
            sc = _dot(q[h], k[h], NT) * (LANES ** -0.5 * LOG2E)
            sc = jnp.where(mask, sc, -1e9 * LOG2E)
            p[h] = jnp.exp2(sc - jnp.max(sc, axis=1, keepdims=True))
            l[h] = jnp.sum(p[h], axis=1, keepdims=True)

        def values(h):
            inv = pl.reciprocal(l[h], approx=True)
            inv = inv * (2.0 - l[h] * inv)
            ob_v[:, h * LANES:(h + 1) * LANES] = _dot(p[h], v[h]) * inv

        def out_proj(g):
            for n in range(n_col):
                w = pltpu.bitcast(wo_v[n, g * 256:(g + 1) * 256, :], BF16)
                r = _dot(ob_v[:, g * 512:(g + 1) * 512], w)
                acc[n] = r if acc[n] is None else acc[n] + r

        n_grp = n_head // GROUP
        todo = list(range(n_head // 4))
        for i in range(n_grp + 2):
            if i < n_grp:
                for h in range(i * GROUP, (i + 1) * GROUP):
                    proj(h)
            else:
                for _ in range(3):
                    out_proj(todo.pop(0))
            if i == 0:
                finish(s - 1, jnp.maximum(s - 1, 0))
            if i == n_grp:
                norm_live(jnp.minimum(s + 1, n_seg - 1))
            if 1 <= i <= n_grp:
                for h in range((i - 1) * GROUP, i * GROUP):
                    scores(h)
            if i >= 2:
                for h in range((i - 2) * GROUP, (i - 1) * GROUP):
                    values(h)
        while todo:
            out_proj(todo.pop(0))
        o = jnp.concatenate(acc, axis=1)
        att_v[...] = o[n_mem:]
        return o[:n_mem]

    lax.fori_loop(0, n_seg, seg_body, mem_v[...].astype(F32))

    finish(n_seg - 1, n_seg - 1)
    cp_out1.start()

    r = r_v[...] + 0.0
    bits = pltpu.bitcast(r, I32)
    key = jnp.where(bits < 0, bits ^ 0x7FFFFFFF, bits)
    key = jnp.where(r != r, INT_MIN + 1, key)
    key = jnp.where(seg_lane < n_seg, key, INT_MIN)
    pos = seg_lane * seg + lax.broadcasted_iota(I32, (seg, LANES), 0)

    def best(key):
        top = jnp.max(jnp.max(key, axis=0, keepdims=True), axis=1, keepdims=True)
        cand = jnp.where(key == top, pos, n_seg * seg - 1)
        return jnp.min(jnp.min(cand, axis=0, keepdims=True), axis=1, keepdims=True)

    v0 = best(key)
    v1 = best(jnp.where(pos == v0, INT_MIN, key))
    i0, i1 = v0[0, 0], v1[0, 0]

    sub = lax.broadcasted_iota(I32, (8, d_model), 0)
    h = jnp.where(sub == 0, h_v[pl.ds(i0, 1), :], h_v[pl.ds(i1, 1), :])
    hn = _layernorm(h)
    gate = _rb(jax.nn.sigmoid(_rb(jnp.sum(hn * wr_v[...].astype(F32), axis=-1, keepdims=True))))
    cp_wg.wait()
    cp_wu.wait()
    cp_wd.wait()
    g = _rb(_dot(hn, wg_v[...]))
    u = _rb(_dot(hn, wu_v[...]))
    a = _rb(_rb(g * jax.nn.sigmoid(g)) * u)
    y = _rb(_rb(_dot(a, wd_v[...])) * gate)
    new = h + _rb(hn + y)

    s0, s1 = i0 // seg, i1 // seg
    tok = lax.broadcasted_iota(I32, (seg, d_model), 0)
    for slot, sg in enumerate((s0, s1)):
        blk = out_v[sg].astype(F32)
        blk = jnp.where(tok == i0 - sg * seg, new[0:1], blk)
        blk = jnp.where(tok == i1 - sg * seg, new[1:2], blk)
        patch_v[slot] = blk.astype(BF16)
    cp_out0.wait()
    cp_out1.wait()
    cp_p0 = pltpu.make_async_copy(patch_v.at[0], out_hbm.at[s0], sem.at[9])
    cp_p1 = pltpu.make_async_copy(patch_v.at[1], out_hbm.at[s1], sem.at[10])
    cp_p0.start()

    @pl.when(s0 != s1)
    def _():
        cp_p1.start()
        cp_p1.wait()

    cp_p0.wait()


@functools.partial(jax.jit, static_argnames=("A_seg_len",))
def pallas_sequential_preLN__memory_aug_recurrent_mem_tr__moe_arch_mod__prompt_kernel(
    A_x: jax.Array,
    A_mem0: jax.Array,
    A_Wq: jax.Array,
    A_Wk: jax.Array,
    A_Wv: jax.Array,
    A_Wo: jax.Array,
    A_seg_len: int,
    B_x: jax.Array,
    B_w_r: jax.Array,
    B_w_gate: jax.Array,
    B_w_up: jax.Array,
    B_w_down: jax.Array,
):
    del B_x
    batch, seq, d_model = A_x.shape
    _, n_head, d_head = A_Wq.shape
    n_mem = A_mem0.shape[1]
    d_ff = B_w_gate.shape[1]
    seg = int(A_seg_len)
    n_seg = seq // seg
    assert batch == 1 and d_head == LANES and n_seg * seg == seq and n_seg <= LANES

    kernel = functools.partial(_kernel, n_seg=n_seg, seg=seg, n_mem=n_mem,
                               n_head=n_head, d_model=d_model)
    out = pl.pallas_call(
        kernel,
        out_shape=jax.ShapeDtypeStruct((n_seg, seg, d_model), A_x.dtype),
        in_specs=[pl.BlockSpec(memory_space=pl.ANY)] * 10,
        out_specs=pl.BlockSpec(memory_space=pl.ANY),
        scratch_shapes=[
            pltpu.VMEM((n_seg, seg, d_model), BF16),
            pltpu.VMEM((n_seg, PRE, d_model), BF16),
            pltpu.VMEM((n_seg * PRE, d_model), BF16),
            pltpu.VMEM((3, n_head // 2, d_model, LANES), U32),
            pltpu.VMEM((3, n_head, d_model // 2, LANES), U32),
            pltpu.VMEM((d_model // LANES, n_head * LANES // 2, LANES), U32),
            pltpu.VMEM((3, n_head, n_seg * PRE, LANES), F32),
            pltpu.VMEM((n_mem, d_model), BF16),
            pltpu.VMEM((1, d_model), BF16),
            pltpu.VMEM((d_model, d_ff), BF16),
            pltpu.VMEM((d_model, d_ff), BF16),
            pltpu.VMEM((d_ff, d_model), BF16),
            pltpu.VMEM((n_mem + seg, n_head * LANES), F32),
            pltpu.VMEM((seg - PRE, d_model), F32),
            pltpu.VMEM((seg, d_model), F32),
            pltpu.VMEM((seq, d_model), F32),
            pltpu.VMEM((n_seg, seg, d_model), BF16),
            pltpu.VMEM((seg, LANES), F32),
            pltpu.VMEM((2, seg, d_model), BF16),
            pltpu.SemaphoreType.DMA((3, n_head // 2)),
            pltpu.SemaphoreType.DMA((16,)),
        ],
        compiler_params=pltpu.CompilerParams(vmem_limit_bytes=100 * 1024 * 1024),
        name="rmt_mod_block",
    )(A_x.reshape(n_seg, seg, d_model), A_mem0.reshape(n_mem, d_model), A_Wq, A_Wk, A_Wv,
      A_Wo.reshape(n_head * d_head, d_model), B_w_r.reshape(1, d_model), B_w_gate, B_w_up,
      B_w_down)
    return out.reshape(batch, seq, d_model)
```

```python
import functools
import math

import jax
import jax.numpy as jnp
import numpy as np
from jax import lax
from jax.experimental import pallas as pl
from jax.experimental.pallas import tpu as pltpu

F32, BF16, U32, I32 = jnp.float32, jnp.bfloat16, jnp.uint32, jnp.int32
NN = (((1,), (0,)), ((), ()))
NT = (((1,), (1,)), ((), ()))
LANES = 128
PRE = 8
GROUP = 4
EPS_BF16 = float(np.float32(1e-05).astype(BF16))
LOG2E = math.log2(math.e)
INT_MIN = int(np.iinfo(np.int32).min)


def _rb(x):
    return x.astype(BF16).astype(F32)


def _layernorm(x):
    inv_n = 1.0 / x.shape[-1]
    m = jnp.sum(x, axis=-1, keepdims=True) * inv_n
    c = x - m
    v = _rb(jnp.sum(c * c, axis=-1, keepdims=True) * inv_n)
    d = _rb(jnp.sqrt(_rb(v + EPS_BF16)))
    return _rb(_rb(x - _rb(m)) * (1.0 / d))


def _dot(a, b, dims=NN):
    return lax.dot_general(a, b, dims, preferred_element_type=F32)


def _kernel(x_hbm, mem_hbm, wq_hbm, wk_hbm, wv_hbm, wo_hbm, wr_hbm, wg_hbm,
            wu_hbm, wd_hbm, out_hbm,
            x_v, xpre_v, lpre_v, raw_v, w_v, wo_v, pre_v, mem_v, wr_v, wg_v,
            wu_v, wd_v, ob_v, xn_v, att_v, h_v, out_v, r_v, patch_v,
            sem_raw, sem, *, n_seg, seg, n_mem, n_head, d_model):
    live = seg - PRE
    rows = n_mem + seg
    n_pair = n_head // 2
    n_col = d_model // LANES
    w_hbms = (wq_hbm, wk_hbm, wv_hbm)

    def raw_copy(t, j):
        return pltpu.make_async_copy(
            w_hbms[t].bitcast(U32).at[:, j, :], raw_v.at[t, j], sem_raw.at[t, j])

    cp_xpre = pltpu.make_async_copy(x_hbm.at[:, pl.ds(live, PRE), :], xpre_v, sem.at[0])
    cp_mem = pltpu.make_async_copy(mem_hbm, mem_v, sem.at[1])
    cp_wr = pltpu.make_async_copy(wr_hbm, wr_v, sem.at[2])
    cp_x = pltpu.make_async_copy(x_hbm, x_v, sem.at[3])
    cp_wg = pltpu.make_async_copy(wg_hbm, wg_v, sem.at[4])
    cp_wu = pltpu.make_async_copy(wu_hbm, wu_v, sem.at[5])
    cp_wd = pltpu.make_async_copy(wd_hbm, wd_v, sem.at[6])
    cp_wo = [pltpu.make_async_copy(
        wo_hbm.bitcast(U32).at[:, pl.ds(n * LANES, LANES)], wo_v.at[n], sem.at[11 + n])
        for n in range(n_col)]

    cp_xpre.start()
    for t in range(3):
        raw_copy(t, 0).start()
    cp_mem.start()
    cp_wr.start()

    cp_xpre.wait()
    for t in range(3):
        raw_copy(t, 1).start()
    xp = xpre_v[...].astype(F32).reshape(n_seg * PRE, d_model)
    lpre_v[...] = _layernorm(xp).astype(BF16)

    def pro_body(j, carry):
        for t in range(3):
            raw_copy(t, j).wait()

        @pl.when(j + 2 < n_pair)
        def _():
            for t in range(3):
                raw_copy(t, j + 2).start()

        for n, c in enumerate(cp_wo + [cp_x]):
            pl.when(j == 4 + 2 * n)(c.start)

        for t in range(3):
            a = raw_v[t, j, pl.ds(0, d_model // 2, stride=2), :]
            b = raw_v[t, j, pl.ds(1, d_model // 2, stride=2), :]
            for p, w in enumerate(((a & 0xFFFF) | (b << 16),
                                   (a >> 16) | (b & np.uint32(0xFFFF0000)))):
                w_v[t, 2 * j + p] = w
                pre_v[t, 2 * j + p] = _dot(lpre_v[...], pltpu.bitcast(w, BF16))
        return carry

    lax.fori_loop(0, n_pair, pro_body, 0)

    cp_mem.wait()
    cp_wr.wait()
    cp_x.wait()
    for c in cp_wo:
        c.wait()
    cp_wg.start()
    cp_wu.start()
    cp_wd.start()

    def norm_live(s):
        xn_v[...] = _layernorm(x_v[s].astype(F32)[:live])

    seg_lane = lax.broadcasted_iota(I32, (seg, LANES), 1)

    def finish(s, slot):
        h = _rb(x_v[slot].astype(F32) + _rb(att_v[...]))
        hn = _layernorm(h)
        h_v[pl.ds(pl.multiple_of(slot * seg, seg), seg), :] = h
        out_v[slot] = (h + hn).astype(BF16)
        wr = wr_v[...].astype(F32)
        r = _rb(jnp.sum(hn * wr, axis=-1, keepdims=True))
        r_v[...] = jnp.where(seg_lane == s, r, r_v[...])

    norm_live(0)
    att_v[...] = jnp.zeros_like(att_v)
    r_v[...] = jnp.zeros_like(r_v)

    row = lax.broadcasted_iota(I32, (rows, rows), 0)
    col = lax.broadcasted_iota(I32, (rows, rows), 1)
    mask = (row < n_mem) | (row >= col)
    cut = n_seg - 8
    cp_out0 = pltpu.make_async_copy(out_v.at[pl.ds(0, cut)], out_hbm.at[pl.ds(0, cut)], sem.at[7])
    cp_out1 = pltpu.make_async_copy(out_v.at[pl.ds(cut, n_seg - cut)],
                                    out_hbm.at[pl.ds(cut, n_seg - cut)], sem.at[8])

    def seg_body(s, mem):
        @pl.when(s == cut + 1)
        def _():
            cp_out0.start()

        lhs = jnp.concatenate([mem, xn_v[...]], axis=0).astype(BF16)
        pre_rows = pl.ds(pl.multiple_of(s * PRE, PRE), PRE)
        q, k, v, p, l = {}, {}, {}, {}, {}
        acc = [None] * n_col

        def proj(h):
            for t, dst in enumerate((q, k, v)):
                dst[h] = jnp.concatenate(
                    [_dot(lhs, pltpu.bitcast(w_v[t, h], BF16)), pre_v[t, h, pre_rows, :]], axis=0)

        def scores(h):
            sc = _dot(q[h], k[h], NT) * (LANES ** -0.5 * LOG2E)
            sc = jnp.where(mask, sc, -1e9 * LOG2E)
            p[h] = jnp.exp2(sc - jnp.max(sc, axis=1, keepdims=True))
            l[h] = jnp.sum(p[h], axis=1, keepdims=True)

        def values(h):
            inv = pl.reciprocal(l[h], approx=True)
            inv = inv * (2.0 - l[h] * inv)
            ob_v[:, h * LANES:(h + 1) * LANES] = _dot(p[h], v[h]) * inv

        def out_proj(g):
            for n in range(n_col):
                w = pltpu.bitcast(wo_v[n, g * 256:(g + 1) * 256, :], BF16)
                r = _dot(ob_v[:, g * 512:(g + 1) * 512], w)
                acc[n] = r if acc[n] is None else acc[n] + r

        n_grp = n_head // GROUP
        todo = list(range(n_head // 4))
        for i in range(n_grp + 2):
            if i < n_grp:
                for h in range(i * GROUP, (i + 1) * GROUP):
                    proj(h)
            else:
                for _ in range(3):
                    out_proj(todo.pop(0))
            if i == 0:
                finish(s - 1, jnp.maximum(s - 1, 0))
            if i == n_grp:
                norm_live(jnp.minimum(s + 1, n_seg - 1))
            if 1 <= i <= n_grp:
                for h in range((i - 1) * GROUP, i * GROUP):
                    scores(h)
            if i >= 2:
                for h in range((i - 2) * GROUP, (i - 1) * GROUP):
                    values(h)
        while todo:
            out_proj(todo.pop(0))
        o = jnp.concatenate(acc, axis=1)
        att_v[...] = o[n_mem:]
        return o[:n_mem]

    lax.fori_loop(0, n_seg, seg_body, mem_v[...].astype(F32))

    finish(n_seg - 1, n_seg - 1)
    cp_out1.start()

    r = r_v[...] + 0.0
    bits = pltpu.bitcast(r, I32)
    key = jnp.where(bits < 0, bits ^ 0x7FFFFFFF, bits)
    key = jnp.where(r != r, INT_MIN + 1, key)
    key = jnp.where(seg_lane < n_seg, key, INT_MIN)
    pos = seg_lane * seg + lax.broadcasted_iota(I32, (seg, LANES), 0)

    def best(key):
        top = jnp.max(jnp.max(key, axis=0, keepdims=True), axis=1, keepdims=True)
        cand = jnp.where(key == top, pos, n_seg * seg - 1)
        return jnp.min(jnp.min(cand, axis=0, keepdims=True), axis=1, keepdims=True)

    v0 = best(key)
    v1 = best(jnp.where(pos == v0, INT_MIN, key))
    i0, i1 = v0[0, 0], v1[0, 0]

    sub = lax.broadcasted_iota(I32, (8, d_model), 0)
    h = jnp.where(sub == 0, h_v[pl.ds(i0, 1), :], h_v[pl.ds(i1, 1), :])
    hn = _layernorm(h)
    gate = _rb(jax.nn.sigmoid(_rb(jnp.sum(hn * wr_v[...].astype(F32), axis=-1, keepdims=True))))
    cp_wg.wait()
    cp_wu.wait()
    cp_wd.wait()
    g = _rb(_dot(hn, wg_v[...]))
    u = _rb(_dot(hn, wu_v[...]))
    a = _rb(_rb(g * jax.nn.sigmoid(g)) * u)
    y = _rb(_rb(_dot(a, wd_v[...])) * gate)
    new = h + _rb(hn + y)

    s0, s1 = i0 // seg, i1 // seg
    tok = lax.broadcasted_iota(I32, (seg, d_model), 0)
    for slot, sg in enumerate((s0, s1)):
        blk = out_v[sg].astype(F32)
        blk = jnp.where(tok == i0 - sg * seg, new[0:1], blk)
        blk = jnp.where(tok == i1 - sg * seg, new[1:2], blk)
        patch_v[slot] = blk.astype(BF16)
    cp_out0.wait()
    cp_out1.wait()
    cp_p0 = pltpu.make_async_copy(patch_v.at[0], out_hbm.at[s0], sem.at[9])
    cp_p1 = pltpu.make_async_copy(patch_v.at[1], out_hbm.at[s1], sem.at[10])
    cp_p0.start()

    @pl.when(s0 != s1)
    def _():
        cp_p1.start()
        cp_p1.wait()

    cp_p0.wait()


@functools.partial(jax.jit, static_argnames=("A_seg_len",))
def pallas_sequential_preLN__memory_aug_recurrent_mem_tr__moe_arch_mod__prompt_kernel(
    A_x: jax.Array,
    A_mem0: jax.Array,
    A_Wq: jax.Array,
    A_Wk: jax.Array,
    A_Wv: jax.Array,
    A_Wo: jax.Array,
    A_seg_len: int,
    B_x: jax.Array,
    B_w_r: jax.Array,
    B_w_gate: jax.Array,
    B_w_up: jax.Array,
    B_w_down: jax.Array,
):
    del B_x
    batch, seq, d_model = A_x.shape
    _, n_head, d_head = A_Wq.shape
    n_mem = A_mem0.shape[1]
    d_ff = B_w_gate.shape[1]
    seg = int(A_seg_len)
    n_seg = seq // seg
    assert batch == 1 and d_head == LANES and n_seg * seg == seq and n_seg <= LANES

    kernel = functools.partial(_kernel, n_seg=n_seg, seg=seg, n_mem=n_mem,
                               n_head=n_head, d_model=d_model)
    out = pl.pallas_call(
        kernel,
        out_shape=jax.ShapeDtypeStruct((n_seg, seg, d_model), A_x.dtype),
        in_specs=[pl.BlockSpec(memory_space=pl.ANY)] * 10,
        out_specs=pl.BlockSpec(memory_space=pl.ANY),
        scratch_shapes=[
            pltpu.VMEM((n_seg, seg, d_model), BF16),
            pltpu.VMEM((n_seg, PRE, d_model), BF16),
            pltpu.VMEM((n_seg * PRE, d_model), BF16),
            pltpu.VMEM((3, n_head // 2, d_model, LANES), U32),
            pltpu.VMEM((3, n_head, d_model // 2, LANES), U32),
            pltpu.VMEM((d_model // LANES, n_head * LANES // 2, LANES), U32),
            pltpu.VMEM((3, n_head, n_seg * PRE, LANES), F32),
            pltpu.VMEM((n_mem, d_model), BF16),
            pltpu.VMEM((1, d_model), BF16),
            pltpu.VMEM((d_model, d_ff), BF16),
            pltpu.VMEM((d_model, d_ff), BF16),
            pltpu.VMEM((d_ff, d_model), BF16),
            pltpu.VMEM((n_mem + seg, n_head * LANES), F32),
            pltpu.VMEM((seg - PRE, d_model), F32),
            pltpu.VMEM((seg, d_model), F32),
            pltpu.VMEM((seq, d_model), F32),
            pltpu.VMEM((n_seg, seg, d_model), BF16),
            pltpu.VMEM((seg, LANES), F32),
            pltpu.VMEM((2, seg, d_model), BF16),
            pltpu.SemaphoreType.DMA((3, n_head // 2)),
            pltpu.SemaphoreType.DMA((16,)),
        ],
        compiler_params=pltpu.CompilerParams(vmem_limit_bytes=100 * 1024 * 1024),
        name="rmt_mod_block",
    )(A_x.reshape(n_seg, seg, d_model), A_mem0.reshape(n_mem, d_model), A_Wq, A_Wk, A_Wv,
      A_Wo.reshape(n_head * d_head, d_model), B_w_r.reshape(1, d_model), B_w_gate, B_w_up,
      B_w_down)
    return out.reshape(batch, seq, d_model)
```

```python
import functools
import math

import jax
import jax.numpy as jnp
import numpy as np
from jax import lax
from jax.experimental import pallas as pl
from jax.experimental.pallas import tpu as pltpu

F32, BF16, U32, I32 = jnp.float32, jnp.bfloat16, jnp.uint32, jnp.int32
NN = (((1,), (0,)), ((), ()))
NT = (((1,), (1,)), ((), ()))
LANES = 128
PRE = 8
GROUP = 4
UNROLL = 4
EARLY = 8
LATE_G = 4
BATCHES = (2, 3, 5, 8, 13, 17)
XBLK = 8
EPS_BF16 = float(np.float32(1e-05).astype(BF16))
LOG2E = math.log2(math.e)
INT_MIN = int(np.iinfo(np.int32).min)


def _rb(x):
    return x.astype(BF16).astype(F32)


def _layernorm(x):
    inv_n = 1.0 / x.shape[-1]
    m = jnp.sum(x, axis=-1, keepdims=True) * inv_n
    c = x - m
    v = _rb(jnp.sum(c * c, axis=-1, keepdims=True) * inv_n)
    d = _rb(jnp.sqrt(_rb(v + EPS_BF16)))
    return _rb(_rb(x - _rb(m)) * (1.0 / d))


def _dot(a, b, dims=NN):
    return lax.dot_general(a, b, dims, preferred_element_type=F32)


def _sort_key(r):
    bits = pltpu.bitcast(r, I32)
    key = jnp.where(bits < 0, bits ^ 0x7FFFFFFF, bits)
    key = jnp.where(r == 0.0, 0, key)
    return jnp.where(r != r, INT_MIN + 1, key)


def _kernel(x_hbm, mem_hbm, wq_hbm, wk_hbm, wv_hbm, wo_hbm, wr_hbm, wg_hbm,
            wu_hbm, wd_hbm, out_hbm,
            x_v, xpre_v, lpre_v, raw_v, w_v, wo_v, pre_v, mem_v, wr_v, wrf_v, wg_v,
            wu_v, wd_v, ob_v, xn_v, att_v, h_v, hn_v, out_v, top_v, patch_v,
            sem_raw, sem_x, sem_wo, sem, *, n_seg, seg, n_mem, n_head, d_model):
    live = seg - PRE
    rows = n_mem + seg
    n_pair = n_head // 2
    n_col = d_model // LANES
    w_hbms = (wq_hbm, wk_hbm, wv_hbm)
    blk_seg = n_seg // XBLK
    blk = blk_seg * PRE

    def raw_copy(t, j):
        return pltpu.make_async_copy(
            w_hbms[t].bitcast(U32).at[:, j, :], raw_v.at[t, j], sem_raw.at[t, j])

    cp_xpre = pltpu.make_async_copy(x_hbm.at[:, pl.ds(live, PRE), :], xpre_v, sem_x.at[0])
    cp_mem = pltpu.make_async_copy(mem_hbm, mem_v, sem.at[0])
    cp_wr = pltpu.make_async_copy(wr_hbm, wr_v, sem.at[1])
    cp_x = pltpu.make_async_copy(x_hbm, x_v, sem.at[2])
    cp_wg = pltpu.make_async_copy(wg_hbm, wg_v, sem.at[3])
    cp_wu = pltpu.make_async_copy(wu_hbm, wu_v, sem.at[4])
    cp_wd = pltpu.make_async_copy(wd_hbm, wd_v, sem.at[5])
    cp_wo = [pltpu.make_async_copy(
        wo_hbm.bitcast(U32).at[:, pl.ds(n * LANES, LANES)], wo_v.at[n], sem_wo.at[n])
        for n in range(n_col)]

    def repack(t, j):
        a = raw_v[t, j, pl.ds(0, d_model // 2, stride=2), :]
        b = raw_v[t, j, pl.ds(1, d_model // 2, stride=2), :]
        w_v[t, 2 * j] = (a & 0xFFFF) | (b << 16)
        w_v[t, 2 * j + 1] = (a >> 16) | (b & np.uint32(0xFFFF0000))

    def pre_project(t, h, lo, n):
        pre_v[t, h, lo:lo + n, :] = _dot(lpre_v[lo:lo + n, :], pltpu.bitcast(w_v[t, h], BF16))

    units = [(t, j) for j in range(n_pair) for t in range(3)]
    edges = np.cumsum((0,) + BATCHES)
    assert edges[-1] == len(units)
    batches = [units[a:b] for a, b in zip(edges[:-1], edges[1:])]
    cp_xpre.start()
    for u in batches[0]:
        raw_copy(*u).start()
    cp_xpre.wait()
    for i, batch in enumerate(batches):
        for u in batch:
            raw_copy(*u).wait()
        if i + 1 < len(batches):
            for u in batches[i + 1]:
                raw_copy(*u).start()
        else:
            for c in [cp_mem, cp_wr, cp_x] + cp_wo:
                c.start()
        if i == 0:
            for t, j in batch:
                repack(t, j)
            for b in range(XBLK):
                xp = xpre_v[b * blk_seg:(b + 1) * blk_seg].astype(F32).reshape(blk, d_model)
                lpre_v[b * blk:(b + 1) * blk, :] = _layernorm(xp).astype(BF16)
                for t, j in batch:
                    pre_project(t, 2 * j, b * blk, blk)
                    pre_project(t, 2 * j + 1, b * blk, blk)
        else:
            for t, j in batch:
                repack(t, j)
                pre_project(t, 2 * j, 0, n_seg * PRE)
                pre_project(t, 2 * j + 1, 0, n_seg * PRE)

    cp_mem.wait()
    cp_wr.wait()
    cp_x.wait()
    for c in cp_wo:
        c.wait()
    cp_wg.start()
    cp_wu.start()
    cp_wd.start()

    sub = lax.broadcasted_iota(I32, (8, LANES), 0)

    def norm_live(s, c):
        xn = _layernorm(x_v[s, 8 * c:8 * c + 8, :].astype(F32))
        xn_v[8 * c:8 * c + 8, :] = xn
        return pltpu.bitcast(xn[:, :LANES], I32)

    def finish(s, slot, c):
        rs = slice(8 * c, 8 * c + 8)
        h = _rb(x_v[slot, rs, :].astype(F32) + _rb(att_v[rs, :]))
        hn = _layernorm(h)
        at = pl.ds(pl.multiple_of(slot * seg + 8 * c, 8), 8)
        h_v[at, :] = h
        hn_v[at, :] = hn
        out_v[slot, rs, :] = (h + hn).astype(BF16)
        r = _rb(jnp.sum(hn * wrf_v[...], axis=-1, keepdims=True))
        key = _sort_key(jnp.broadcast_to(r, (8, LANES)))
        key = jnp.where(s >= 0, key, INT_MIN)
        pos = slot * seg + 8 * c + sub
        k0, p0, k1, p1 = top_v[0], top_v[1], top_v[2], top_v[3]
        first, second = key > k0, key > k1
        k1 = jnp.where(first, k0, jnp.where(second, key, k1))
        top_v[0] = jnp.where(first, key, k0)
        top_v[1] = jnp.where(first, pos, p0)
        top_v[2] = k1
        top_v[3] = jnp.where(first, p0, jnp.where(second, pos, p1))
        return k1

    for c in range(live // 8):
        norm_live(0, c)
    wrf_v[...] = jnp.broadcast_to(wr_v[...].astype(F32).reshape(1, d_model), wrf_v.shape)
    att_v[...] = jnp.zeros_like(att_v)
    for i in range(2):
        top_v[2 * i] = jnp.full((8, LANES), INT_MIN, I32)
        top_v[2 * i + 1] = jnp.zeros((8, LANES), I32)

    row = lax.broadcasted_iota(I32, (rows, rows), 0)
    col = lax.broadcasted_iota(I32, (rows, rows), 1)
    mask = (row < n_mem) | (row >= col)
    cut = n_seg - UNROLL - 1
    cp_out0 = pltpu.make_async_copy(out_v.at[pl.ds(0, cut)], out_hbm.at[pl.ds(0, cut)], sem.at[6])
    cp_out1 = pltpu.make_async_copy(out_v.at[pl.ds(cut, n_seg - cut)],
                                    out_hbm.at[pl.ds(cut, n_seg - cut)], sem.at[7])

    def segment(s, mem, split):
        lhs = [jnp.concatenate([mem[n], xn_v[:, n * LANES:(n + 1) * LANES]], axis=0).astype(BF16)
               for n in range(n_col)]
        pre_rows = pl.ds(pl.multiple_of(s * PRE, PRE), PRE)
        qkv, p, l, part = ({}, {}, {}), {}, {}, {}
        acc = [None] * n_col
        k_cut = (n_col - 1) * LANES // 2

        if split:
            head = jnp.concatenate(lhs[:-1], axis=1)
            for i in range(EARLY):
                t, h = i % 3, i // 3
                part[t, h] = _dot(head, pltpu.bitcast(w_v[t, h, :k_cut, :], BF16))
        full = jnp.concatenate(lhs, axis=1)

        def proj(h):
            for t in range(3):
                if (t, h) in part:
                    r = _dot(lhs[-1], pltpu.bitcast(w_v[t, h, k_cut:, :], BF16)) + part[t, h]
                else:
                    r = _dot(full, pltpu.bitcast(w_v[t, h], BF16))
                qkv[t][h] = jnp.concatenate([r, pre_v[t, h, pre_rows, :]], axis=0)

        def scores(h, after=None):
            sc = _dot(qkv[0][h], qkv[1][h], NT) * (LANES ** -0.5 * LOG2E)
            fill = -1e9 * LOG2E
            if after is not None:
                fill = jnp.where(after[:, :rows] == 1, 0.0, fill)
                fill = jnp.concatenate([fill] * (rows // 8), axis=0)
            sc = jnp.where(mask, sc, fill)
            p[h] = jnp.exp2(sc - jnp.max(sc, axis=1, keepdims=True))
            l[h] = jnp.sum(p[h], axis=1, keepdims=True)

        def values(h):
            inv = pl.reciprocal(l[h], approx=True)
            inv = inv * (2.0 - l[h] * inv)
            ob_v[:, h * LANES:(h + 1) * LANES] = _dot(p[h], qkv[2][h]) * inv

        def out_proj(g, n):
            w = pltpu.bitcast(wo_v[n, g * 256:(g + 1) * 256, :], BF16)
            r = _dot(ob_v[:, g * 512:(g + 1) * 512], w)
            acc[n] = r if acc[n] is None else r + acc[n]

        n_grp = n_head // GROUP
        n_g = n_head // 4
        late = [(g, n_col - 1) for g in range(n_g - LATE_G, n_g)]
        todo = [(g, n) for g in range(n_g) for n in range(n_col) if (g, n) not in late] + late
        side = [functools.partial(finish, s - 1, jnp.maximum(s - 1, 0), c) for c in range(seg // 8)]
        side += [functools.partial(norm_live, jnp.minimum(s + 1, n_seg - 1), c)
                 for c in range(live // 8)]
        for i in range(n_grp + 2):
            if i < n_grp:
                for h in range(i * GROUP, (i + 1) * GROUP):
                    proj(h)
            else:
                for _ in range(10):
                    out_proj(*todo.pop(0))
            if 1 <= i <= n_grp:
                after = side.pop(0)() if i >= 2 and side else None
                for h in range((i - 1) * GROUP, i * GROUP):
                    scores(h, after if h == i * GROUP - 1 else None)
            if i >= 2:
                for h in range((i - 2) * GROUP, (i - 1) * GROUP):
                    values(h)
        assert not side
        while todo:
            out_proj(*todo.pop(0))
        for n in range(n_col):
            att_v[:, n * LANES:(n + 1) * LANES] = acc[n][n_mem:]
        return [a[:n_mem] for a in acc]

    def seg_body(i, mem):
        @pl.when(i == n_seg // UNROLL - 1)
        def _():
            cp_out0.start()

        for u in range(UNROLL):
            mem = segment(i * UNROLL + u, mem, u > 0)
        return mem

    mem0 = mem_v[...].astype(F32)
    lax.fori_loop(0, n_seg // UNROLL, seg_body, [mem0[:, n * LANES:(n + 1) * LANES] for n in range(n_col)])

    cp_wg.wait()
    cp_wu.wait()
    cp_wd.wait()
    for c in range(seg // 8):
        finish(n_seg - 1, n_seg - 1, c)
    cp_out1.start()

    key = jnp.concatenate([top_v[0], top_v[2]], axis=0)
    pos = jnp.concatenate([top_v[1], top_v[3]], axis=0)

    def best(key):
        top = jnp.max(key, axis=0, keepdims=True)
        return jnp.min(jnp.where(key == top, pos, n_seg * seg - 1), axis=0, keepdims=True)

    v0 = best(key)
    v1 = best(jnp.where(pos == v0, INT_MIN, key))
    i0, i1 = v0[0, 0], v1[0, 0]

    first = lax.broadcasted_iota(I32, (8, d_model), 0) == 0
    h = jnp.where(first, h_v[pl.ds(i0, 1), :], h_v[pl.ds(i1, 1), :])
    hn = jnp.where(first, hn_v[pl.ds(i0, 1), :], hn_v[pl.ds(i1, 1), :])
    gate = _rb(jax.nn.sigmoid(_rb(jnp.sum(hn * wrf_v[...], axis=-1, keepdims=True))))
    g = _rb(_dot(hn, wg_v[...]))
    u = _rb(_dot(hn, wu_v[...]))
    a = _rb(_rb(g * jax.nn.sigmoid(g)) * u)
    y = _rb(_rb(_dot(a, wd_v[...])) * gate)
    new = h + _rb(hn + y)

    s0, s1 = i0 // seg, i1 // seg
    tok_w = lax.broadcasted_iota(I32, (seg, d_model), 0)
    for slot, sg in enumerate((s0, s1)):
        o = out_v[sg].astype(F32)
        o = jnp.where(tok_w == i0 - sg * seg, new[0:1], o)
        o = jnp.where(tok_w == i1 - sg * seg, new[1:2], o)
        patch_v[slot] = o.astype(BF16)
    cp_out0.wait()
    cp_out1.wait()
    cp_p0 = pltpu.make_async_copy(patch_v.at[0], out_hbm.at[s0], sem.at[8])
    cp_p1 = pltpu.make_async_copy(patch_v.at[1], out_hbm.at[s1], sem.at[9])
    cp_p0.start()

    @pl.when(s0 != s1)
    def _():
        cp_p1.start()
        cp_p1.wait()

    cp_p0.wait()


@functools.partial(jax.jit, static_argnames=("A_seg_len",))
def pallas_sequential_preLN__memory_aug_recurrent_mem_tr__moe_arch_mod__prompt_kernel(
    A_x: jax.Array,
    A_mem0: jax.Array,
    A_Wq: jax.Array,
    A_Wk: jax.Array,
    A_Wv: jax.Array,
    A_Wo: jax.Array,
    A_seg_len: int,
    B_x: jax.Array,
    B_w_r: jax.Array,
    B_w_gate: jax.Array,
    B_w_up: jax.Array,
    B_w_down: jax.Array,
):
    del B_x
    batch, seq, d_model = A_x.shape
    _, n_head, d_head = A_Wq.shape
    n_mem = A_mem0.shape[1]
    d_ff = B_w_gate.shape[1]
    seg = int(A_seg_len)
    n_seg = seq // seg
    assert batch == 1 and d_head == LANES and n_seg * seg == seq

    kernel = functools.partial(_kernel, n_seg=n_seg, seg=seg, n_mem=n_mem,
                               n_head=n_head, d_model=d_model)
    out = pl.pallas_call(
        kernel,
        out_shape=jax.ShapeDtypeStruct((n_seg, seg, d_model), A_x.dtype),
        in_specs=[pl.BlockSpec(memory_space=pl.ANY)] * 10,
        out_specs=pl.BlockSpec(memory_space=pl.ANY),
        scratch_shapes=[
            pltpu.VMEM((n_seg, seg, d_model), BF16),
            pltpu.VMEM((n_seg, PRE, d_model), BF16),
            pltpu.VMEM((n_seg * PRE, d_model), BF16),
            pltpu.VMEM((3, n_head // 2, d_model, LANES), U32),
            pltpu.VMEM((3, n_head, d_model // 2, LANES), U32),
            pltpu.VMEM((d_model // LANES, n_head * LANES // 2, LANES), U32),
            pltpu.VMEM((3, n_head, n_seg * PRE, LANES), F32),
            pltpu.VMEM((n_mem, d_model), BF16),
            pltpu.VMEM((d_model,), BF16),
            pltpu.VMEM((8, d_model), F32),
            pltpu.VMEM((d_model, d_ff), BF16),
            pltpu.VMEM((d_model, d_ff), BF16),
            pltpu.VMEM((d_ff, d_model), BF16),
            pltpu.VMEM((n_mem + seg, n_head * LANES), F32),
            pltpu.VMEM((seg - PRE, d_model), F32),
            pltpu.VMEM((seg, d_model), F32),
            pltpu.VMEM((seq, d_model), F32),
            pltpu.VMEM((seq, d_model), F32),
            pltpu.VMEM((n_seg, seg, d_model), BF16),
            pltpu.VMEM((4, 8, LANES), I32)  ,
            pltpu.VMEM((2, seg, d_model), BF16),
            pltpu.SemaphoreType.DMA((3, n_head // 2)),
            pltpu.SemaphoreType.DMA((XBLK,)),
            pltpu.SemaphoreType.DMA((d_model // LANES,)),
            pltpu.SemaphoreType.DMA((10,)),
        ],
        compiler_params=pltpu.CompilerParams(vmem_limit_bytes=100 * 1024 * 1024),
        name="rmt_mod_block",
    )(A_x.reshape(n_seg, seg, d_model), A_mem0.reshape(n_mem, d_model), A_Wq, A_Wk, A_Wv,
      A_Wo.reshape(n_head * d_head, d_model), B_w_r, B_w_gate, B_w_up, B_w_down)
    return out.reshape(batch, seq, d_model)
```

```python
import functools
import math

import jax
import jax.numpy as jnp
import numpy as np
from jax import lax
from jax.experimental import pallas as pl
from jax.experimental.pallas import tpu as pltpu

F32, BF16, U32, I32 = jnp.float32, jnp.bfloat16, jnp.uint32, jnp.int32
NN = (((1,), (0,)), ((), ()))
NT = (((1,), (1,)), ((), ()))
LANES = 128
PRE = 8
GROUP = 4
UNROLL = 8
EARLY = 8
LATE_G = 4
BATCHES = (2, 4, 6)
NOBC = True
XBLK = 8
EPS_BF16 = float(np.float32(1e-05).astype(BF16))
LOG2E = math.log2(math.e)
INT_MIN = int(np.iinfo(np.int32).min)


def _rb(x):
    return x.astype(BF16).astype(F32)


def _layernorm(x):
    inv_n = 1.0 / x.shape[-1]
    m = jnp.sum(x, axis=-1, keepdims=True) * inv_n
    c = x - m
    v = _rb(jnp.sum(c * c, axis=-1, keepdims=True) * inv_n)
    d = _rb(jnp.sqrt(_rb(v + EPS_BF16)))
    return _rb(_rb(x - _rb(m)) * (1.0 / d))


def _dot(a, b, dims=NN):
    return lax.dot_general(a, b, dims, preferred_element_type=F32)


def _sort_key(r):
    bits = pltpu.bitcast(r, I32)
    key = jnp.where(bits < 0, bits ^ 0x7FFFFFFF, bits)
    key = jnp.where(r == 0.0, 0, key)
    return jnp.where(r != r, INT_MIN + 1, key)


def _kernel(x_hbm, mem_hbm, wq_hbm, wk_hbm, wv_hbm, wo_hbm, wr_hbm, wg_hbm,
            wu_hbm, wd_hbm, out_hbm,
            x_v, x0_v, xpre_v, lpre_v, raw_v, w_v, wo_v, pre_v, mem_v, wr_v, wrf_v, wg_v,
            wu_v, wd_v, ob_v, xn_v, att_v, h_v, hn_v, out_v, top_v, patch_v,
            sem, *, n_seg, seg, n_mem, n_head, d_model):
    live = seg - PRE
    rows = n_mem + seg
    n_pair = n_head // 2
    n_col = d_model // LANES
    w_hbms = (wq_hbm, wk_hbm, wv_hbm)
    blk_seg = n_seg // XBLK
    blk = blk_seg * PRE

    def raw_copy(t, j):
        return pltpu.make_async_copy(
            w_hbms[t].bitcast(U32).at[:, j, :], raw_v.at[t, j], sem.at[0])

    cp_xpre = pltpu.make_async_copy(x_hbm.at[:, pl.ds(live, PRE), :], xpre_v, sem.at[0])
    cp_mem = pltpu.make_async_copy(mem_hbm, mem_v, sem.at[1])
    cp_wr = pltpu.make_async_copy(wr_hbm, wr_v, sem.at[1])
    cp_x0 = pltpu.make_async_copy(x_hbm.at[0], x0_v, sem.at[1])
    cp_wg = pltpu.make_async_copy(wg_hbm, wg_v, sem.at[0])
    cp_wu = pltpu.make_async_copy(wu_hbm, wu_v, sem.at[0])
    cp_wd = pltpu.make_async_copy(wd_hbm, wd_v, sem.at[0])

    def wo_copy(n):
        cols = pl.ds(pl.multiple_of(n * LANES, LANES), LANES)
        return pltpu.make_async_copy(wo_hbm.bitcast(U32).at[:, cols], wo_v.at[n], sem.at[1])

    def x_copy(n):
        part = pl.ds(n * (n_seg // n_col), n_seg // n_col)
        return pltpu.make_async_copy(x_hbm.at[part], x_v.at[part], sem.at[1])

    def repack(t, j):
        a = raw_v[t, j, pl.ds(0, d_model // 2, stride=2), :]
        b = raw_v[t, j, pl.ds(1, d_model // 2, stride=2), :]
        w_v[t, 2 * j] = (a & 0xFFFF) | (b << 16)
        w_v[t, 2 * j + 1] = (a >> 16) | (b & np.uint32(0xFFFF0000))

    def pre_project(t, h, lo, n):
        pre_v[t, h, lo:lo + n, :] = _dot(lpre_v[lo:lo + n, :], pltpu.bitcast(w_v[t, h], BF16))

    units = [(t, j) for j in range(n_pair) for t in range(3)]
    edges = np.cumsum((0,) + BATCHES)
    peeled = int(edges[-1]) // 3
    per_trip = (n_pair - peeled) // n_col
    assert edges[-1] == 3 * peeled and peeled + per_trip * n_col == n_pair
    batches = [units[a:b] for a, b in zip(edges[:-1], edges[1:])]

    def trip_units(n):
        return [(t, peeled + n * per_trip + j) for j in range(per_trip) for t in range(3)]

    def project_units(batch):
        for t, j in batch:
            repack(t, j)
            pre_project(t, 2 * j, 0, n_seg * PRE)
            pre_project(t, 2 * j + 1, 0, n_seg * PRE)

    cp_xpre.start()
    for u in batches[0]:
        raw_copy(*u).start()
    cp_xpre.wait()
    for i, batch in enumerate(batches):
        for u in batch:
            raw_copy(*u).wait()
        last = i + 1 == len(batches)
        if last:
            for c in (cp_mem, cp_wr, cp_x0):
                c.wait()
        for u in trip_units(0) if last else batches[i + 1]:
            raw_copy(*u).start()
        if i == 0:
            for c in (cp_mem, cp_wr, cp_x0):
                c.start()
            for t, j in batch:
                repack(t, j)
            for b in range(XBLK):
                xp = xpre_v[b * blk_seg:(b + 1) * blk_seg].astype(F32).reshape(blk, d_model)
                lpre_v[b * blk:(b + 1) * blk, :] = _layernorm(xp).astype(BF16)
                for t, j in batch:
                    pre_project(t, 2 * j, b * blk, blk)
                    pre_project(t, 2 * j + 1, b * blk, blk)
        else:
            project_units(batch)
        if last:
            xn_v[...] = _layernorm(x0_v[:live, :].astype(F32))
            wrf_v[...] = jnp.broadcast_to(wr_v[...].astype(F32).reshape(1, d_model), wrf_v.shape)
            att_v[...] = jnp.zeros_like(att_v)
            for n in range(2):
                top_v[2 * n] = jnp.full((8, LANES), INT_MIN, I32)
                top_v[2 * n + 1] = jnp.zeros((8, LANES), I32)

    def pro_body(n, carry):
        wo_copy(n).start()
        x_copy(n).start()
        for u in trip_units(n):
            raw_copy(*u).wait()

        @pl.when(n + 1 < n_col)
        def _():
            for u in trip_units(n + 1):
                raw_copy(*u).start()

        project_units(trip_units(n))
        return carry

    lax.fori_loop(0, n_col, pro_body, 0)

    for n in range(n_col):
        wo_copy(n).wait()
        x_copy(n).wait()
    cp_wg.start()
    cp_wu.start()
    cp_wd.start()

    sub = lax.broadcasted_iota(I32, (8, LANES), 0)

    def norm_live(s, c):
        xn = _layernorm(x_v[s, 8 * c:8 * c + 8, :].astype(F32))
        xn_v[8 * c:8 * c + 8, :] = xn
        return pltpu.bitcast(xn[:, :LANES], I32)

    def finish(s, slot, c):
        rs = slice(8 * c, 8 * c + 8)
        h = _rb(x_v[slot, rs, :].astype(F32) + _rb(att_v[rs, :]))
        hn = _layernorm(h)
        at = pl.ds(pl.multiple_of(slot * seg + 8 * c, 8), 8)
        h_v[at, :] = h
        hn_v[at, :] = hn
        out_v[slot, rs, :] = (h + hn).astype(BF16)
        r = _rb(jnp.sum(hn * wrf_v[...], axis=-1, keepdims=True))
        key = _sort_key(jnp.broadcast_to(r, (8, LANES)))
        key = jnp.where(s >= 0, key, INT_MIN)
        pos = slot * seg + 8 * c + sub
        k0, p0, k1, p1 = top_v[0], top_v[1], top_v[2], top_v[3]
        first, second = key > k0, key > k1
        k1 = jnp.where(first, k0, jnp.where(second, key, k1))
        top_v[0] = jnp.where(first, key, k0)
        top_v[1] = jnp.where(first, pos, p0)
        top_v[2] = k1
        top_v[3] = jnp.where(first, p0, jnp.where(second, pos, p1))
        return k1

    row = lax.broadcasted_iota(I32, (rows, rows), 0)
    col = lax.broadcasted_iota(I32, (rows, rows), 1)
    mask = (row < n_mem) | (row >= col)
    cut = n_seg - UNROLL - 1
    cp_out0 = pltpu.make_async_copy(out_v.at[pl.ds(0, cut)], out_hbm.at[pl.ds(0, cut)], sem.at[1])
    cp_out1 = pltpu.make_async_copy(out_v.at[pl.ds(cut, n_seg - cut)],
                                    out_hbm.at[pl.ds(cut, n_seg - cut)], sem.at[1])

    def segment(s, mem, split):
        lhs = [jnp.concatenate([mem[n], xn_v[:, n * LANES:(n + 1) * LANES]], axis=0).astype(BF16)
               for n in range(n_col)]
        pre_rows = pl.ds(pl.multiple_of(s * PRE, PRE), PRE)
        qkv, p, l, part = ({}, {}, {}), {}, {}, {}
        acc = [None] * n_col
        k_cut = (n_col - 1) * LANES // 2

        if split:
            head = jnp.concatenate(lhs[:-1], axis=1)
            for i in range(EARLY):
                t, h = i % 3, i // 3
                part[t, h] = _dot(head, pltpu.bitcast(w_v[t, h, :k_cut, :], BF16))
        full = jnp.concatenate(lhs, axis=1)

        def proj(h):
            for t in range(3):
                if (t, h) in part:
                    r = _dot(lhs[-1], pltpu.bitcast(w_v[t, h, k_cut:, :], BF16)) + part[t, h]
                else:
                    r = _dot(full, pltpu.bitcast(w_v[t, h], BF16))
                qkv[t][h] = jnp.concatenate([r, pre_v[t, h, pre_rows, :]], axis=0)

        def scores(h, after=None):
            sc = _dot(qkv[0][h], qkv[1][h], NT) * (LANES ** -0.5 * LOG2E)
            fill = -1e9 * LOG2E
            if after is not None:
                fill = jnp.where(after[:, :rows] == 1, 0.0, fill)
                fill = jnp.concatenate([fill] * (rows // 8), axis=0)
            sc = jnp.where(mask, sc, fill)
            p[h] = jnp.exp2(sc - jnp.max(sc, axis=1, keepdims=True))
            l[h] = jnp.sum(p[h], axis=1, keepdims=True)

        def values(h):
            inv = pl.reciprocal(l[h], approx=True)
            inv = inv * (2.0 - l[h] * inv)
            ob_v[:, h * LANES:(h + 1) * LANES] = _dot(p[h], qkv[2][h]) * inv

        def out_proj(g, n):
            w = pltpu.bitcast(wo_v[n, g * 256:(g + 1) * 256, :], BF16)
            r = _dot(ob_v[:, g * 512:(g + 1) * 512], w)
            acc[n] = r if acc[n] is None else r + acc[n]

        n_grp = n_head // GROUP
        n_g = n_head // 4
        late = [(g, n_col - 1) for g in range(n_g - LATE_G, n_g)]
        todo = [(g, n) for g in range(n_g) for n in range(n_col) if (g, n) not in late] + late
        side = [functools.partial(finish, s - 1, jnp.maximum(s - 1, 0), c) for c in range(seg // 8)]
        side += [functools.partial(norm_live, jnp.minimum(s + 1, n_seg - 1), c)
                 for c in range(live // 8)]
        for i in range(n_grp + 2):
            if i < n_grp:
                for h in range(i * GROUP, (i + 1) * GROUP):
                    proj(h)
            else:
                for _ in range(10):
                    out_proj(*todo.pop(0))
            if 1 <= i <= n_grp:
                after = side.pop(0)() if i >= 2 and side else None
                for h in range((i - 1) * GROUP, i * GROUP):
                    scores(h, after if h == i * GROUP - 1 else None)
            if i >= 2:
                for h in range((i - 2) * GROUP, (i - 1) * GROUP):
                    values(h)
        assert not side
        while todo:
            out_proj(*todo.pop(0))
        for n in range(n_col):
            att_v[:, n * LANES:(n + 1) * LANES] = acc[n][n_mem:]
        return [a[:n_mem] for a in acc]

    def seg_body(i, mem):
        @pl.when(i == n_seg // UNROLL - 1)
        def _():
            cp_out0.start()

        for u in range(UNROLL):
            mem = segment(i * UNROLL + u, mem, u > 0)
        return mem

    mem0 = mem_v[...].astype(F32)
    lax.fori_loop(0, n_seg // UNROLL, seg_body, [mem0[:, n * LANES:(n + 1) * LANES] for n in range(n_col)])

    for c in range(seg // 8):
        finish(n_seg - 1, n_seg - 1, c)
    cp_out1.start()

    key = jnp.concatenate([top_v[0], top_v[2]], axis=0)
    pos = jnp.concatenate([top_v[1], top_v[3]], axis=0)

    def best(key):
        top = jnp.max(key, axis=0, keepdims=True)
        return jnp.min(jnp.where(key == top, pos, n_seg * seg - 1), axis=0, keepdims=True)

    v0 = best(key)
    v1 = best(jnp.where(pos == v0, INT_MIN, key))
    i0, i1 = v0[0, 0], v1[0, 0]
    cp_wg.wait()
    cp_wu.wait()
    cp_wd.wait()

    first = lax.broadcasted_iota(I32, (8, d_model), 0) == 0
    h = jnp.where(first, h_v[pl.ds(i0, 1), :], h_v[pl.ds(i1, 1), :])
    hn = jnp.where(first, hn_v[pl.ds(i0, 1), :], hn_v[pl.ds(i1, 1), :])
    gate = _rb(jax.nn.sigmoid(_rb(jnp.sum(hn * wrf_v[...], axis=-1, keepdims=True))))
    g = _rb(_dot(hn, wg_v[...]))
    u = _rb(_dot(hn, wu_v[...]))
    a = _rb(_rb(g * jax.nn.sigmoid(g)) * u)
    y = _rb(_rb(_dot(a, wd_v[...])) * gate)
    new = h + _rb(hn + y)

    base = [pl.multiple_of(i & -8, 8) for i in (i0, i1)]
    tok = lax.broadcasted_iota(I32, (8, d_model), 0)
    for slot, b in enumerate(base):
        o = h_v[pl.ds(b, 8), :] + hn_v[pl.ds(b, 8), :]
        o = jnp.where(tok == i0 - b, new[0:1], o)
        o = jnp.where(tok == i1 - b, new[1:2], o)
        patch_v[slot] = o.astype(BF16)
    cp_out0.wait()
    cp_out1.wait()
    cp_p0, cp_p1 = (pltpu.make_async_copy(
        patch_v.at[slot],
        out_hbm.at[lax.div(b, seg), pl.ds(pl.multiple_of(lax.rem(b, seg), 8), 8), :],
        sem.at[slot]) for slot, b in enumerate(base))
    cp_p0.start()

    @pl.when(base[0] != base[1])
    def _():
        cp_p1.start()
        cp_p1.wait()

    cp_p0.wait()


@functools.partial(jax.jit, static_argnames=("A_seg_len",))
def pallas_sequential_preLN__memory_aug_recurrent_mem_tr__moe_arch_mod__prompt_kernel(
    A_x: jax.Array,
    A_mem0: jax.Array,
    A_Wq: jax.Array,
    A_Wk: jax.Array,
    A_Wv: jax.Array,
    A_Wo: jax.Array,
    A_seg_len: int,
    B_x: jax.Array,
    B_w_r: jax.Array,
    B_w_gate: jax.Array,
    B_w_up: jax.Array,
    B_w_down: jax.Array,
):
    del B_x
    batch, seq, d_model = A_x.shape
    _, n_head, d_head = A_Wq.shape
    n_mem = A_mem0.shape[1]
    d_ff = B_w_gate.shape[1]
    seg = int(A_seg_len)
    n_seg = seq // seg
    assert batch == 1 and d_head == LANES and n_seg * seg == seq

    kernel = functools.partial(_kernel, n_seg=n_seg, seg=seg, n_mem=n_mem,
                               n_head=n_head, d_model=d_model)
    out = pl.pallas_call(
        kernel,
        out_shape=jax.ShapeDtypeStruct((n_seg, seg, d_model), A_x.dtype),
        in_specs=[pl.BlockSpec(memory_space=pl.ANY)] * 10,
        out_specs=pl.BlockSpec(memory_space=pl.ANY),
        scratch_shapes=[
            pltpu.VMEM((n_seg, seg, d_model), BF16),
            pltpu.VMEM((seg, d_model), BF16),
            pltpu.VMEM((n_seg, PRE, d_model), BF16),
            pltpu.VMEM((n_seg * PRE, d_model), BF16),
            pltpu.VMEM((3, n_head // 2, d_model, LANES), U32),
            pltpu.VMEM((3, n_head, d_model // 2, LANES), U32),
            pltpu.VMEM((d_model // LANES, n_head * LANES // 2, LANES), U32),
            pltpu.VMEM((3, n_head, n_seg * PRE, LANES), F32),
            pltpu.VMEM((n_mem, d_model), BF16),
            pltpu.VMEM((d_model,), BF16),
            pltpu.VMEM((8, d_model), F32),
            pltpu.VMEM((d_model, d_ff), BF16),
            pltpu.VMEM((d_model, d_ff), BF16),
            pltpu.VMEM((d_ff, d_model), BF16),
            pltpu.VMEM((n_mem + seg, n_head * LANES), F32),
            pltpu.VMEM((seg - PRE, d_model), F32),
            pltpu.VMEM((seg, d_model), F32),
            pltpu.VMEM((seq, d_model), F32),
            pltpu.VMEM((seq, d_model), F32),
            pltpu.VMEM((n_seg, seg, d_model), BF16),
            pltpu.VMEM((4, 8, LANES), I32)  ,
            pltpu.VMEM((2, 8, d_model), BF16),
            pltpu.SemaphoreType.DMA((2,)),
        ],
        compiler_params=pltpu.CompilerParams(vmem_limit_bytes=100 * 1024 * 1024,
                                             disable_bounds_checks=NOBC),
        name="rmt_mod_block",
    )(A_x.reshape(n_seg, seg, d_model), A_mem0.reshape(n_mem, d_model), A_Wq, A_Wk, A_Wv,
      A_Wo.reshape(n_head * d_head, d_model), B_w_r, B_w_gate, B_w_up, B_w_down)
    return out.reshape(batch, seq, d_model)
```

```python
import functools
import math

import jax
import jax.numpy as jnp
import numpy as np
from jax import lax
from jax.experimental import pallas as pl
from jax.experimental.pallas import tpu as pltpu

F32, BF16, U32, I32 = jnp.float32, jnp.bfloat16, jnp.uint32, jnp.int32
NN = (((1,), (0,)), ((), ()))
NT = (((1,), (1,)), ((), ()))
LANES = 128
PRE = 8
BATCHES = (2, 4, 6)
XBLK = 8
UNROLL = 8
GROUP = 4
OUT_STEP = 10
LATE = 4
EARLY = 8
EPS_BF16 = float(np.float32(1e-05).astype(BF16))
LOG2E = math.log2(math.e)
INT_MIN = int(np.iinfo(np.int32).min)


def _rb(x):
    return x.astype(BF16).astype(F32)


def _layernorm(x):
    inv_n = 1.0 / x.shape[-1]
    m = jnp.sum(x, axis=-1, keepdims=True) * inv_n
    c = x - m
    v = _rb(jnp.sum(c * c, axis=-1, keepdims=True) * inv_n)
    d = _rb(jnp.sqrt(_rb(v + EPS_BF16)))
    return _rb(_rb(x - _rb(m)) * (1.0 / d))


def _dot(a, b, dims=NN):
    return lax.dot_general(a, b, dims, preferred_element_type=F32)


def _sort_key(r):
    bits = pltpu.bitcast(r, I32)
    key = jnp.where(bits < 0, bits ^ 0x7FFFFFFF, bits)
    key = jnp.where(r == 0.0, 0, key)
    return jnp.where(r != r, INT_MIN + 1, key)


def _kernel(x_hbm, mem_hbm, wq_hbm, wk_hbm, wv_hbm, wo_hbm, wr_hbm, wg_hbm,
            wu_hbm, wd_hbm, out_hbm,
            x_v, x0_v, xpre_v, lpre_v, raw_v, w_v, wo_v, pre_v, mem_v, wr_v,
            wrf_v, wg_v, wu_v, wd_v, ob_v, xn_v, att_v, h_v, hn_v, out_v, top_v,
            patch_v, sem, *, n_seg, seg, n_mem, n_head, d_model):
    live = seg - PRE
    rows = n_mem + seg
    n_pair = n_head // 2
    n_col = d_model // LANES
    n_pre = n_seg * PRE
    cols = [slice(n * LANES, (n + 1) * LANES) for n in range(n_col)]

    def raw_copy(t, j):
        src = (wq_hbm, wk_hbm, wv_hbm)[t].bitcast(U32).at[:, j, :]
        return pltpu.make_async_copy(src, raw_v.at[t, j], sem.at[0])

    def wo_copy(n):
        src = wo_hbm.bitcast(U32).at[:, pl.ds(pl.multiple_of(n * LANES, LANES), LANES)]
        return pltpu.make_async_copy(src, wo_v.at[n], sem.at[1])

    def x_copy(n):
        part = pl.ds(n * (n_seg // n_col), n_seg // n_col)
        return pltpu.make_async_copy(x_hbm.at[part], x_v.at[part], sem.at[1])

    def out_copy(lo, hi):
        part = pl.ds(lo, hi - lo)
        return pltpu.make_async_copy(out_v.at[part], out_hbm.at[part], sem.at[1])

    cp_xpre = pltpu.make_async_copy(x_hbm.at[:, pl.ds(live, PRE), :], xpre_v, sem.at[0])
    cp_small = [pltpu.make_async_copy(src, dst, sem.at[1]) for src, dst in
                ((mem_hbm, mem_v), (wr_hbm, wr_v), (x_hbm.at[0], x0_v))]
    cp_ffn = [pltpu.make_async_copy(src, dst, sem.at[0]) for src, dst in
              ((wg_hbm, wg_v), (wu_hbm, wu_v), (wd_hbm, wd_v))]

    def repack(t, j):
        even = raw_v[t, j, pl.ds(0, d_model // 2, stride=2), :]
        odd = raw_v[t, j, pl.ds(1, d_model // 2, stride=2), :]
        w_v[t, 2 * j] = (even & 0xFFFF) | (odd << 16)
        w_v[t, 2 * j + 1] = (even >> 16) | (odd & np.uint32(0xFFFF0000))

    def pre_project(t, j, rs):
        for h in (2 * j, 2 * j + 1):
            pre_v[t, h, rs, :] = _dot(lpre_v[rs, :], pltpu.bitcast(w_v[t, h], BF16))

    def project_units(batch):
        for t, j in batch:
            repack(t, j)
            pre_project(t, j, slice(0, n_pre))

    units = [(t, j) for j in range(n_pair) for t in range(3)]
    edges = [sum(BATCHES[:i]) for i in range(len(BATCHES) + 1)]
    batches = [units[a:b] for a, b in zip(edges[:-1], edges[1:])]
    peeled = edges[-1] // 3
    per_trip = (n_pair - peeled) // n_col
    assert edges[-1] == 3 * peeled and peeled + per_trip * n_col == n_pair

    def trip_units(n):
        return [(t, peeled + n * per_trip + j) for j in range(per_trip) for t in range(3)]

    cp_xpre.start()
    for u in batches[0]:
        raw_copy(*u).start()
    cp_xpre.wait()
    for i, batch in enumerate(batches):
        last = i + 1 == len(batches)
        for u in batch:
            raw_copy(*u).wait()
        if last:
            for c in cp_small:
                c.wait()
        for u in trip_units(0) if last else batches[i + 1]:
            raw_copy(*u).start()
        if i == 0:
            for c in cp_small:
                c.start()
            for t, j in batch:
                repack(t, j)
            for b in range(XBLK):
                lo, hi = b * n_seg // XBLK, (b + 1) * n_seg // XBLK
                rs = slice(lo * PRE, hi * PRE)
                xp = xpre_v[lo:hi].astype(F32).reshape((hi - lo) * PRE, d_model)
                lpre_v[rs, :] = _layernorm(xp).astype(BF16)
                for t, j in batch:
                    pre_project(t, j, rs)
        else:
            project_units(batch)
    xn_v[...] = _layernorm(x0_v[:live, :].astype(F32))
    wrf_v[...] = jnp.broadcast_to(wr_v[...].astype(F32).reshape(1, d_model), wrf_v.shape)
    att_v[...] = jnp.zeros_like(att_v)
    for n in range(2):
        top_v[2 * n] = jnp.full((8, LANES), INT_MIN, I32)
        top_v[2 * n + 1] = jnp.zeros((8, LANES), I32)

    def pro_body(n, carry):
        wo_copy(n).start()
        x_copy(n).start()
        for u in trip_units(n):
            raw_copy(*u).wait()

        @pl.when(n + 1 < n_col)
        def _():
            for u in trip_units(n + 1):
                raw_copy(*u).start()

        project_units(trip_units(n))
        return carry

    lax.fori_loop(0, n_col, pro_body, 0)
    for n in range(n_col):
        wo_copy(n).wait()
        x_copy(n).wait()
    for c in cp_ffn:
        c.start()

    sub = lax.broadcasted_iota(I32, (8, LANES), 0)
    row = lax.broadcasted_iota(I32, (rows, rows), 0)
    col = lax.broadcasted_iota(I32, (rows, rows), 1)
    mask = (row < n_mem) | (row >= col)

    def norm_live(s, c):
        xn = _layernorm(x_v[s, 8 * c:8 * c + 8, :].astype(F32))
        xn_v[8 * c:8 * c + 8, :] = xn
        return pltpu.bitcast(xn[:, :LANES], I32)

    def finish(s, slot, c):
        rs = slice(8 * c, 8 * c + 8)
        h = _rb(x_v[slot, rs, :].astype(F32) + _rb(att_v[rs, :]))
        hn = _layernorm(h)
        at = pl.ds(pl.multiple_of(slot * seg + 8 * c, 8), 8)
        h_v[at, :] = h
        hn_v[at, :] = hn
        out_v[slot, rs, :] = (h + hn).astype(BF16)
        r = _rb(jnp.sum(hn * wrf_v[...], axis=-1, keepdims=True))
        key = _sort_key(jnp.broadcast_to(r, (8, LANES)))
        key = jnp.where(s >= 0, key, INT_MIN)
        pos = slot * seg + 8 * c + sub
        k0, p0, k1, p1 = top_v[0], top_v[1], top_v[2], top_v[3]
        first, second = key > k0, key > k1
        k1 = jnp.where(first, k0, jnp.where(second, key, k1))
        top_v[0] = jnp.where(first, key, k0)
        top_v[1] = jnp.where(first, pos, p0)
        top_v[2] = k1
        top_v[3] = jnp.where(first, p0, jnp.where(second, pos, p1))
        return k1

    def segment(s, mem, split):
        lhs = [jnp.concatenate([mem[n], xn_v[:, cols[n]]], axis=0).astype(BF16)
               for n in range(n_col)]
        pre_rows = pl.ds(pl.multiple_of(s * PRE, PRE), PRE)
        qkv, p, l, part = ({}, {}, {}), {}, {}, {}
        acc = [None] * n_col
        k_cut = (n_col - 1) * LANES // 2
        if split:
            head = jnp.concatenate(lhs[:-1], axis=1)
            for i in range(EARLY):
                t, h = i % 3, i // 3
                part[t, h] = _dot(head, pltpu.bitcast(w_v[t, h, :k_cut, :], BF16))
        full = jnp.concatenate(lhs, axis=1)

        def proj(h):
            for t in range(3):
                if (t, h) in part:
                    r = _dot(lhs[-1], pltpu.bitcast(w_v[t, h, k_cut:, :], BF16)) + part[t, h]
                else:
                    r = _dot(full, pltpu.bitcast(w_v[t, h], BF16))
                r = jnp.concatenate([r, pre_v[t, h, pre_rows, :]], axis=0)
                qkv[t][h] = r.astype(BF16) if t else r

        def scores(h, after):
            sc = _dot(qkv[0][h], qkv[1][h], NT) * (LANES ** -0.5 * LOG2E)
            fill = -1e9 * LOG2E
            if after is not None:
                fill = jnp.where(after[:, :rows] == 1, 0.0, fill)
                fill = jnp.concatenate([fill] * (rows // 8), axis=0)
            sc = jnp.where(mask, sc, fill)
            p[h] = jnp.exp2(sc - jnp.max(sc, axis=1, keepdims=True))
            l[h] = jnp.sum(p[h], axis=1, keepdims=True)

        def values(h):
            inv = pl.reciprocal(l[h], approx=True)
            inv = inv * (2.0 - l[h] * inv)
            ob_v[:, h * LANES:(h + 1) * LANES] = _dot(p[h], qkv[2][h]) * inv

        def out_proj(g, n):
            lo, hi = g * GROUP * LANES, (g + 1) * GROUP * LANES
            r = _dot(ob_v[:, lo:hi], pltpu.bitcast(wo_v[n, lo // 2:hi // 2, :], BF16))
            acc[n] = r if acc[n] is None else r + acc[n]

        n_grp = n_head // GROUP
        late = [(g, n_col - 1) for g in range(n_grp - LATE, n_grp)]
        todo = [(g, n) for g in range(n_grp) for n in range(n_col) if (g, n) not in late] + late
        side = [functools.partial(finish, s - 1, jnp.maximum(s - 1, 0), c)
                for c in range(seg // 8)]
        side += [functools.partial(norm_live, jnp.minimum(s + 1, n_seg - 1), c)
                 for c in range(live // 8)]
        for i in range(n_grp + 2):
            if i < n_grp:
                for h in range(i * GROUP, (i + 1) * GROUP):
                    proj(h)
            else:
                for _ in range(OUT_STEP):
                    g, n = todo.pop(0)
                    assert g < i - 2
                    out_proj(g, n)
            if 1 <= i <= n_grp:
                after = side.pop(0)() if i >= 2 and side else None
                for h in range((i - 1) * GROUP, i * GROUP):
                    scores(h, after if h == i * GROUP - 1 else None)
            if i >= 2:
                for h in range((i - 2) * GROUP, (i - 1) * GROUP):
                    values(h)
        assert not side
        for g, n in todo:
            out_proj(g, n)
        for n in range(n_col):
            att_v[:, cols[n]] = acc[n][n_mem:]
        return [a[:n_mem] for a in acc]

    cut = n_seg - UNROLL - 1

    def seg_body(i, mem):
        @pl.when(i == n_seg // UNROLL - 1)
        def _():
            out_copy(0, cut).start()

        for u in range(UNROLL):
            mem = segment(i * UNROLL + u, mem, u > 0)
        return mem

    mem0 = mem_v[...].astype(F32)
    lax.fori_loop(0, n_seg // UNROLL, seg_body, [mem0[:, c] for c in cols])

    for c in range(seg // 8):
        finish(n_seg - 1, n_seg - 1, c)
    out_copy(cut, n_seg).start()

    key = jnp.concatenate([top_v[0], top_v[2]], axis=0)
    pos = jnp.concatenate([top_v[1], top_v[3]], axis=0)

    def best(key):
        top = jnp.max(key, axis=0, keepdims=True)
        return jnp.min(jnp.where(key == top, pos, n_seg * seg - 1), axis=0, keepdims=True)

    v0 = best(key)
    v1 = best(jnp.where(pos == v0, INT_MIN, key))
    i0, i1 = v0[0, 0], v1[0, 0]
    for c in cp_ffn:
        c.wait()

    tok = lax.broadcasted_iota(I32, (8, d_model), 0)
    h = jnp.where(tok == 0, h_v[pl.ds(i0, 1), :], h_v[pl.ds(i1, 1), :])
    hn = jnp.where(tok == 0, hn_v[pl.ds(i0, 1), :], hn_v[pl.ds(i1, 1), :])
    gate = _rb(jax.nn.sigmoid(_rb(jnp.sum(hn * wrf_v[...], axis=-1, keepdims=True))))
    g = _rb(_dot(hn, wg_v[...]))
    u = _rb(_dot(hn, wu_v[...]))
    a = _rb(_rb(g * jax.nn.sigmoid(g)) * u)
    y = _rb(_rb(_dot(a, wd_v[...])) * gate)
    new = h + _rb(hn + y)

    base = [pl.multiple_of(i & -8, 8) for i in (i0, i1)]
    for slot, b in enumerate(base):
        o = h_v[pl.ds(b, 8), :] + hn_v[pl.ds(b, 8), :]
        o = jnp.where(tok == i0 - b, new[0:1], o)
        o = jnp.where(tok == i1 - b, new[1:2], o)
        patch_v[slot] = o.astype(BF16)
    out_copy(0, cut).wait()
    out_copy(cut, n_seg).wait()
    cp_p0, cp_p1 = (pltpu.make_async_copy(
        patch_v.at[slot],
        out_hbm.at[lax.div(b, seg), pl.ds(pl.multiple_of(lax.rem(b, seg), 8), 8), :],
        sem.at[slot]) for slot, b in enumerate(base))
    cp_p0.start()

    @pl.when(base[0] != base[1])
    def _():
        cp_p1.start()
        cp_p1.wait()

    cp_p0.wait()


@functools.partial(jax.jit, static_argnames=("A_seg_len",))
def pallas_sequential_preLN__memory_aug_recurrent_mem_tr__moe_arch_mod__prompt_kernel(
    A_x: jax.Array,
    A_mem0: jax.Array,
    A_Wq: jax.Array,
    A_Wk: jax.Array,
    A_Wv: jax.Array,
    A_Wo: jax.Array,
    A_seg_len: int,
    B_x: jax.Array,
    B_w_r: jax.Array,
    B_w_gate: jax.Array,
    B_w_up: jax.Array,
    B_w_down: jax.Array,
):
    del B_x
    batch, seq, d_model = A_x.shape
    _, n_head, d_head = A_Wq.shape
    n_mem = A_mem0.shape[1]
    d_ff = B_w_gate.shape[1]
    seg = int(A_seg_len)
    n_seg = seq // seg
    assert batch == 1 and d_head == LANES and A_x.dtype == BF16
    assert n_seg * seg == seq and n_seg % UNROLL == 0

    kernel = functools.partial(_kernel, n_seg=n_seg, seg=seg, n_mem=n_mem,
                               n_head=n_head, d_model=d_model)
    out = pl.pallas_call(
        kernel,
        out_shape=jax.ShapeDtypeStruct((n_seg, seg, d_model), A_x.dtype),
        in_specs=[pl.BlockSpec(memory_space=pl.ANY)] * 10,
        out_specs=pl.BlockSpec(memory_space=pl.ANY),
        scratch_shapes=[
            pltpu.VMEM((n_seg, seg, d_model), BF16),
            pltpu.VMEM((seg, d_model), BF16),
            pltpu.VMEM((n_seg, PRE, d_model), BF16),
            pltpu.VMEM((n_seg * PRE, d_model), BF16),
            pltpu.VMEM((3, n_head // 2, d_model, LANES), U32),
            pltpu.VMEM((3, n_head, d_model // 2, LANES), U32),
            pltpu.VMEM((d_model // LANES, n_head * LANES // 2, LANES), U32),
            pltpu.VMEM((3, n_head, n_seg * PRE, LANES), F32),
            pltpu.VMEM((n_mem, d_model), BF16),
            pltpu.VMEM((d_model,), BF16),
            pltpu.VMEM((8, d_model), F32),
            pltpu.VMEM((d_model, d_ff), BF16),
            pltpu.VMEM((d_model, d_ff), BF16),
            pltpu.VMEM((d_ff, d_model), BF16),
            pltpu.VMEM((n_mem + seg, n_head * LANES), F32),
            pltpu.VMEM((seg - PRE, d_model), F32),
            pltpu.VMEM((seg, d_model), F32),
            pltpu.VMEM((seq, d_model), F32),
            pltpu.VMEM((seq, d_model), F32),
            pltpu.VMEM((n_seg, seg, d_model), BF16),
            pltpu.VMEM((4, 8, LANES), I32),
            pltpu.VMEM((2, 8, d_model), BF16),
            pltpu.SemaphoreType.DMA((2,)),
        ],
        compiler_params=pltpu.CompilerParams(vmem_limit_bytes=100 * 1024 * 1024,
                                             disable_bounds_checks=True),
        name="rmt_mod_block",
    )(A_x.reshape(n_seg, seg, d_model), A_mem0.reshape(n_mem, d_model), A_Wq, A_Wk, A_Wv,
      A_Wo.reshape(n_head * d_head, d_model), B_w_r, B_w_gate, B_w_up, B_w_down)
    return out.reshape(batch, seq, d_model)
```
